```python
import jax
import jax.numpy as jnp

def _softmax(x, axis=-1):
    return jax.nn.softmax(x, axis=axis)

def _gelu(x):
    return jax.nn.gelu(x, approximate=True)

def _silu(x):
    return jax.nn.silu(x)

def _sigmoid(x):
    return jax.nn.sigmoid(x)

def _layernorm(x, axis=-1, eps=1e-05):
    m = jnp.mean(x, axis=axis, keepdims=True)
    v = jnp.var(x, axis=axis, keepdims=True)
    return (x - m) / jnp.sqrt(v + eps)

def _scatter_add(tgt, idx, src, axis=0):
    return tgt.at[idx].add(src)

def _segment_sum(src, seg, n):
    return jax.ops.segment_sum(src, seg, n)

class _Rng:

    def __init__(self, key):
        self._k = key

    def _next(self):
        self._k, sub = jax.random.split(self._k)
        return sub

    def normal(self, shape):
        return jax.random.normal(self._next(), shape, dtype=jnp.bfloat16)

    def randint(self, lo, hi, shape):
        return jax.random.randint(self._next(), shape, lo, hi, dtype=jnp.int32)

    def uniform(self, shape, lo=0.0, hi=1.0):
        return jax.random.uniform(self._next(), shape, jnp.bfloat16, lo, hi)

    def permutation(self, n):
        return jax.random.permutation(self._next(), n)
kernel_name = 'adaLN_cond__sliding_block_cached__dense_activation_gelu__decode'

def setup_inputs():
    _rng = _Rng(jax.random.key(int.from_bytes(__import__("os").urandom(4), "little")))
    _w = lambda a: (lambda t: t.astype(jnp.bfloat16) if jnp.issubdtype(t.dtype, jnp.floating) else t)(jnp.asarray(a))

    def _A_setup():
        B, Sq, D = (4, 1, 640)
        Hq, Hkv, Sk, Dh = (32, 32, 8192, 128)
        assert Hq % Hkv == 0, (Hq, Hkv)
        return {'x': _w((lambda *s: _rng.normal(s) * 0.05)(B, Sq, D)), 'k_cache': _w((lambda *s: _rng.normal(s) * 0.05)(B, Hkv, Sk, Dh)), 'v_cache': _w((lambda *s: _rng.normal(s) * 0.05)(B, Hkv, Sk, Dh)), 'wq': _w((lambda *s: _rng.normal(s) * 0.05)(D, Hq * Dh) * D ** (-0.5)), 'wo': _w((lambda *s: _rng.normal(s) * 0.05)(Hq * Dh, D) * (Hq * Dh) ** (-0.5))}
    _A_in = _A_setup()

    def _B_setup():
        B, S, D, F = (4, 1, 640, 1728)
        return {'x': _w((lambda *s: _rng.normal(s) * 0.05)(B, S, D)), 'w1': _w((lambda *s: _rng.normal(s) * 0.05)(D, F) * D ** (-0.5)), 'b1': _w((lambda *s: _rng.normal(s) * 0.05)(F) * 0.01), 'w2': _w((lambda *s: _rng.normal(s) * 0.05)(F, D) * F ** (-0.5)), 'b2': _w((lambda *s: _rng.normal(s) * 0.05)(D) * 0.01)}
    _B_in = _B_setup()
    return {'A_x': _A_in['x'], 'A_k_cache': _A_in['k_cache'], 'A_v_cache': _A_in['v_cache'], 'A_wq': _A_in['wq'], 'A_wo': _A_in['wo'], 'B_x': _B_in['x'], 'B_w1': _B_in['w1'], 'B_b1': _B_in['b1'], 'B_w2': _B_in['w2'], 'B_b2': _B_in['b2'], 'c': _w((lambda *s: _rng.normal(s) * 0.05)(4, 640)), 'w_mod': _w((lambda *s: _rng.normal(s) * 0.05)(640, 6 * 640) * 640 ** (-0.5))}

def reference(A_x, A_k_cache, A_v_cache, A_wq, A_wo, B_x, B_w1, B_b1, B_w2, B_b2, c, w_mod):

    def _A_ref(x, k_cache, v_cache, wq, wo):
        B, Sq, D = x.shape
        Hq, Dh = (32, 128)
        Hkv, Sk = (k_cache.shape[1], k_cache.shape[2])
        W = min(4096, max(256, Sk // 4))
        rep = Hq // Hkv
        q = (lambda x, *d: x.transpose(*d))((x @ wq).reshape(B, Sq, Hq, Dh), 0, 2, 1, 3)
        k = jnp.repeat(k_cache[:, :, Sk - W:, :], rep, axis=1)
        v = jnp.repeat(v_cache[:, :, Sk - W:, :], rep, axis=1)
        scores = jnp.einsum('bhqd,bhkd->bhqk', q, k) * Dh ** (-0.5)
        p = _softmax(scores, axis=-1)
        o = jnp.einsum('bhqk,bhkd->bhqd', p, v)
        return (lambda x, *d: x.transpose(*d))(o, 0, 2, 1, 3).reshape(B, Sq, Hq * Dh) @ wo

    def _B_ref(x, w1, b1, w2, b2):
        h = jnp.einsum('bsd,df->bsf', x, w1) + b1
        h = _gelu(h)
        return jnp.einsum('bsf,fd->bsd', h, w2) + b2
    x = A_x
    mod = (_silu(c) @ w_mod).reshape(c.shape[0], 6, 1, -1)
    sa, ca, ga, sb, cb, gb = (mod[:, 0].copy(), mod[:, 1].copy(), mod[:, 2].copy(), mod[:, 3].copy(), mod[:, 4].copy(), mod[:, 5].copy())
    h = _layernorm(x, axis=-1) * (1 + ca) + sa
    x = x + ga * _A_ref(h, A_k_cache, A_v_cache, A_wq, A_wo)
    h = _layernorm(x, axis=-1) * (1 + cb) + sb
    x = x + gb * _B_ref(h, B_w1, B_b1, B_w2, B_b2)
    return x
```

```python
import jax
import jax.numpy as jnp
import jax.experimental.pallas as pl
import jax.experimental.pallas.tpu as pltpu

_NT = (((1,), (1,)), ((), ()))
_ROWS = 8
_NSLOT = 4
_EPS = 1e-05


def _layernorm(x):
    m = jnp.mean(x, axis=-1, keepdims=True)
    d = x - m
    v = jnp.mean(d * d, axis=-1, keepdims=True)
    return d / jnp.sqrt(v + _EPS)


def _pad_rows(a):
    b, n = a.shape
    return jnp.concatenate([a, jnp.zeros((_ROWS - b, n), a.dtype)], axis=0)


@jax.jit
def pallas_adaLN_cond__sliding_block_cached__dense_activation_gelu__decode_kernel(
    A_x: jax.Array,
    A_k_cache: jax.Array,
    A_v_cache: jax.Array,
    A_wq: jax.Array,
    A_wo: jax.Array,
    B_x: jax.Array,
    B_w1: jax.Array,
    B_b1: jax.Array,
    B_w2: jax.Array,
    B_b2: jax.Array,
    c: jax.Array,
    w_mod: jax.Array,
):
    del B_x
    B, Sq, D = A_x.shape
    _, H, Sk, Dh = A_k_cache.shape
    F = B_w1.shape[1]
    W = min(4096, max(256, Sk // 4))
    S0 = Sk - W
    assert Sq == 1 and B <= _ROWS and A_wq.shape[1] == H * Dh
    bf = A_k_cache.dtype
    f32 = jnp.float32
    scale = Dh ** (-0.5)
    w2_edges = list(range(0, F, 512)) + [F]
    n_w2 = len(w2_edges) - 1

    def kernel(x_hbm, c_hbm, b1_hbm, b2_hbm, k_hbm, v_hbm, wq_hbm, wo_hbm,
               w1t_hbm, w2_hbm, wm_hbm, o_ref,
               x_v, c_v, b1_v, b2_v, kbuf, vbuf, wq_v, wo_v, w1t_v, w2_v, wm_v,
               q_s, acc_s, sem, ksem, vsem):

        def kv_copy(hbm, buf, sems, h, slot):
            return pltpu.make_async_copy(
                hbm.at[:, h, pl.ds(S0, W), :], buf.at[slot], sems.at[slot])

        def cols(ref, a, b):
            return ref.at[:, pl.ds(a, b - a)]

        cp_c = pltpu.make_async_copy(c_hbm, c_v, sem.at[0])
        cp_wma = pltpu.make_async_copy(
            cols(wm_hbm, 0, 2 * D), cols(wm_v, 0, 2 * D), sem.at[1])
        cp_x = pltpu.make_async_copy(x_hbm, x_v, sem.at[2])
        cp_wq = pltpu.make_async_copy(wq_hbm, wq_v, sem.at[3])
        cp_wo = pltpu.make_async_copy(wo_hbm, wo_v, sem.at[4])
        cp_wmb = pltpu.make_async_copy(
            cols(wm_hbm, 2 * D, 6 * D), cols(wm_v, 2 * D, 6 * D), sem.at[5])
        cp_b1 = pltpu.make_async_copy(b1_hbm, b1_v, sem.at[6])
        cp_b2 = pltpu.make_async_copy(b2_hbm, b2_v, sem.at[7])
        cp_w1 = pltpu.make_async_copy(w1t_hbm, w1t_v, sem.at[8])
        cp_w2 = [
            pltpu.make_async_copy(
                w2_hbm.at[pl.ds(a, b - a), :], w2_v.at[pl.ds(a, b - a), :],
                sem.at[9 + i])
            for i, (a, b) in enumerate(zip(w2_edges[:-1], w2_edges[1:]))
        ]

        cp_wma.start()
        cp_c.start()
        cp_x.start()
        cp_wq.start()
        cp_wo.start()
        for h in range(_NSLOT):
            kv_copy(k_hbm, kbuf, ksem, h, h).start()
            kv_copy(v_hbm, vbuf, vsem, h, h).start()

        cp_c.wait()
        cf = _pad_rows(c_v[...].astype(f32))
        sc = (cf * jax.nn.sigmoid(cf)).astype(bf)
        cp_wma.wait()
        mod_a = jnp.dot(sc, wm_v[:, 0:2 * D], preferred_element_type=f32)
        cp_x.wait()
        x = _pad_rows(x_v[...].astype(f32))
        h_a = _layernorm(x) * (1.0 + mod_a[:, D:2 * D]) + mod_a[:, 0:D]
        cp_wq.wait()
        q = jnp.dot(h_a.astype(bf), wq_v[...], preferred_element_type=f32)
        for h in range(H):
            q_s[h] = q[:, h * Dh:(h + 1) * Dh]
        acc_s[...] = jnp.zeros_like(acc_s)
        cp_wo.wait()

        def head(h, carry):
            slot = h % _NSLOT
            qh = q_s[h].astype(bf)
            row = jax.lax.broadcasted_iota(jnp.int32, (_ROWS, W), 0)
            kv_copy(k_hbm, kbuf, ksem, h, slot).wait()
            s = jnp.zeros((_ROWS, W), f32)
            for b in range(B):
                sb = jax.lax.dot_general(qh, kbuf[slot, b], _NT,
                                         preferred_element_type=f32)
                s = jnp.where(row == b, sb, s)

            @pl.when(h + _NSLOT < H)
            def _():
                kv_copy(k_hbm, kbuf, ksem, h + _NSLOT, slot).start()

            s = s * scale
            e = jnp.exp(s - jnp.max(s, axis=-1, keepdims=True))
            l = jnp.sum(e, axis=-1, keepdims=True)
            p = e.astype(bf)
            row_o = jax.lax.broadcasted_iota(jnp.int32, (_ROWS, Dh), 0)
            kv_copy(v_hbm, vbuf, vsem, h, slot).wait()
            o = jnp.zeros((_ROWS, Dh), f32)
            for b in range(B):
                ob = jnp.dot(p, vbuf[slot, b], preferred_element_type=f32)
                o = jnp.where(row_o == b, ob, o)

            @pl.when(h + _NSLOT < H)
            def _():
                kv_copy(v_hbm, vbuf, vsem, h + _NSLOT, slot).start()

            @pl.when(h + _NSLOT == H)
            def _():
                cp_wmb.start()
                cp_b1.start()
                cp_b2.start()
                cp_w1.start()
                for cp in cp_w2:
                    cp.start()

            o = (o / l).astype(bf)
            wo_h = wo_v[pl.ds(pl.multiple_of(h * Dh, Dh), Dh), :]
            acc_s[...] += jnp.dot(o, wo_h, preferred_element_type=f32)
            return carry

        jax.lax.fori_loop(0, H, head, None)

        cp_wmb.wait()
        mod_b = jnp.dot(sc, wm_v[:, 2 * D:6 * D], preferred_element_type=f32)
        x = x + mod_b[:, 0:D] * acc_s[...]
        h_b = _layernorm(x) * (1.0 + mod_b[:, 2 * D:3 * D]) + mod_b[:, D:2 * D]
        cp_b1.wait()
        cp_b2.wait()
        b1 = b1_v[...].astype(f32).reshape(1, F)
        b2 = b2_v[...].astype(f32).reshape(1, D)
        cp_w1.wait()
        g = jax.lax.dot_general(h_b.astype(bf), w1t_v[...], _NT,
                                preferred_element_type=f32) + b1
        g = jax.nn.gelu(g, approximate=True).astype(bf)
        y = jnp.broadcast_to(b2, (_ROWS, D))
        for cp, a, b in zip(cp_w2, w2_edges[:-1], w2_edges[1:]):
            cp.wait()
            y = y + jnp.dot(g[:, a:b], w2_v[a:b, :], preferred_element_type=f32)
        out = x + mod_b[:, 3 * D:4 * D] * y
        o_ref[...] = out[0:B].astype(o_ref.dtype)

    hbm = pl.BlockSpec(memory_space=pltpu.HBM)
    out = pl.pallas_call(
        kernel,
        out_shape=jax.ShapeDtypeStruct((B, D), A_x.dtype),
        in_specs=[hbm] * 11,
        out_specs=pl.BlockSpec(memory_space=pltpu.VMEM),
        scratch_shapes=[
            pltpu.VMEM((B, D), bf),
            pltpu.VMEM((B, D), bf),
            pltpu.VMEM((F,), bf),
            pltpu.VMEM((D,), bf),
            pltpu.VMEM((_NSLOT, B, W, Dh), bf),
            pltpu.VMEM((_NSLOT, B, W, Dh), bf),
            pltpu.VMEM((D, H * Dh), bf),
            pltpu.VMEM((H * Dh, D), bf),
            pltpu.VMEM((F, D), bf),
            pltpu.VMEM((F, D), bf),
            pltpu.VMEM((D, 6 * D), bf),
            pltpu.VMEM((H, _ROWS, Dh), f32),
            pltpu.VMEM((_ROWS, D), f32),
            pltpu.SemaphoreType.DMA((9 + n_w2,)),
            pltpu.SemaphoreType.DMA((_NSLOT,)),
            pltpu.SemaphoreType.DMA((_NSLOT,)),
        ],
        compiler_params=pltpu.CompilerParams(vmem_limit_bytes=64 * 1024 * 1024),
    )(A_x.reshape(B, D), c, B_b1, B_b2, A_k_cache, A_v_cache, A_wq, A_wo,
      B_w1.T, B_w2, w_mod)
    return out.reshape(B, Sq, D)
```

```python
import jax
import jax.numpy as jnp
import jax.experimental.pallas as pl
import jax.experimental.pallas.tpu as pltpu

_NT = (((1,), (1,)), ((), ()))
_ROWS = 8
_NSLOT = 2
_EPS = 1e-05


def _layernorm(x):
    m = jnp.mean(x, axis=-1, keepdims=True)
    d = x - m
    v = jnp.mean(d * d, axis=-1, keepdims=True)
    return d / jnp.sqrt(v + _EPS)


def _pad_rows(a):
    b, n = a.shape
    return jnp.concatenate([a, jnp.zeros((_ROWS - b, n), a.dtype)], axis=0)


@jax.jit
def pallas_adaLN_cond__sliding_block_cached__dense_activation_gelu__decode_kernel(
    A_x: jax.Array,
    A_k_cache: jax.Array,
    A_v_cache: jax.Array,
    A_wq: jax.Array,
    A_wo: jax.Array,
    B_x: jax.Array,
    B_w1: jax.Array,
    B_b1: jax.Array,
    B_w2: jax.Array,
    B_b2: jax.Array,
    c: jax.Array,
    w_mod: jax.Array,
):
    del B_x
    B, Sq, D = A_x.shape
    _, H, Sk, Dh = A_k_cache.shape
    F = B_w1.shape[1]
    W = min(4096, max(256, Sk // 4))
    S0 = Sk - W
    assert Sq == 1 and B <= _ROWS and A_wq.shape[1] == H * Dh and H >= _NSLOT
    bf = A_k_cache.dtype
    f32 = jnp.float32
    scale = Dh ** (-0.5)
    w2_edges = list(range(0, F, 512)) + [F]
    n_w2 = len(w2_edges) - 1

    def kernel(x_hbm, c_hbm, b1_hbm, b2_hbm, k_hbm, v_hbm, wq_hbm, wo_hbm,
               w1t_hbm, w2_hbm, wm_hbm, o_ref,
               x_v, c_v, b1_v, b2_v, kbuf, vbuf, wq_v, wo_v, w1t_v, w2_v, wm_v,
               q_s, acc_s, sem, ksem, vsem):

        def kv_copy(hbm, buf, sems, h, slot):
            return pltpu.make_async_copy(
                hbm.at[:, h, pl.ds(S0, W), :], buf.at[slot], sems.at[slot])

        cp_c = pltpu.make_async_copy(c_hbm, c_v, sem.at[0])
        cp_wm = pltpu.make_async_copy(wm_hbm, wm_v, sem.at[1])
        cp_x = pltpu.make_async_copy(x_hbm, x_v, sem.at[2])
        cp_wq = pltpu.make_async_copy(wq_hbm, wq_v, sem.at[3])
        cp_wo = pltpu.make_async_copy(wo_hbm, wo_v, sem.at[4])
        cp_b1 = pltpu.make_async_copy(b1_hbm, b1_v, sem.at[5])
        cp_b2 = pltpu.make_async_copy(b2_hbm, b2_v, sem.at[6])
        cp_w1 = pltpu.make_async_copy(w1t_hbm, w1t_v, sem.at[7])
        cp_w2 = [
            pltpu.make_async_copy(
                w2_hbm.at[pl.ds(a, b - a), :], w2_v.at[pl.ds(a, b - a), :],
                sem.at[8 + i])
            for i, (a, b) in enumerate(zip(w2_edges[:-1], w2_edges[1:]))
        ]

        cp_wm.start()
        cp_c.start()
        cp_x.start()
        cp_wq.start()
        cp_wo.start()
        for h in range(_NSLOT):
            kv_copy(k_hbm, kbuf, ksem, h, h).start()
            kv_copy(v_hbm, vbuf, vsem, h, h).start()

        cp_c.wait()
        cf = _pad_rows(c_v[...].astype(f32))
        sc = (cf * jax.nn.sigmoid(cf)).astype(bf)
        cp_wm.wait()
        mod_a = jnp.dot(sc, wm_v[:, 0:2 * D], preferred_element_type=f32)
        cp_x.wait()
        x = _pad_rows(x_v[...].astype(f32))
        h_a = _layernorm(x) * (1.0 + mod_a[:, D:2 * D]) + mod_a[:, 0:D]
        cp_wq.wait()
        q = jnp.dot(h_a.astype(bf), wq_v[...], preferred_element_type=f32)
        for h in range(H):
            q_s[h] = q[:, h * Dh:(h + 1) * Dh]
        acc_s[...] = jnp.zeros_like(acc_s)
        cp_wo.wait()

        def head(h, carry):
            slot = h % _NSLOT
            qh = q_s[h].astype(bf)
            row = jax.lax.broadcasted_iota(jnp.int32, (_ROWS, W), 0)
            kv_copy(k_hbm, kbuf, ksem, h, slot).wait()
            s = jnp.zeros((_ROWS, W), f32)
            for b in range(B):
                sb = jax.lax.dot_general(qh, kbuf[slot, b], _NT,
                                         preferred_element_type=f32)
                s = jnp.where(row == b, sb, s)

            @pl.when(h + _NSLOT < H)
            def _():
                kv_copy(k_hbm, kbuf, ksem, h + _NSLOT, slot).start()

            s = s * scale
            e = jnp.exp(s - jnp.max(s, axis=-1, keepdims=True))
            l = jnp.sum(e, axis=-1, keepdims=True)
            p = e.astype(bf)
            row_o = jax.lax.broadcasted_iota(jnp.int32, (_ROWS, Dh), 0)
            kv_copy(v_hbm, vbuf, vsem, h, slot).wait()
            o = jnp.zeros((_ROWS, Dh), f32)
            for b in range(B):
                ob = jnp.dot(p, vbuf[slot, b], preferred_element_type=f32)
                o = jnp.where(row_o == b, ob, o)

            @pl.when(h + _NSLOT < H)
            def _():
                kv_copy(v_hbm, vbuf, vsem, h + _NSLOT, slot).start()

            @pl.when(h + _NSLOT == H)
            def _():
                cp_b1.start()
                cp_b2.start()
                cp_w1.start()
                for cp in cp_w2:
                    cp.start()

            o = (o / l).astype(bf)
            wo_h = wo_v[pl.ds(pl.multiple_of(h * Dh, Dh), Dh), :]
            acc_s[...] += jnp.dot(o, wo_h, preferred_element_type=f32)
            return carry

        jax.lax.fori_loop(0, H, head, None)

        mod_b = jnp.dot(sc, wm_v[:, 2 * D:6 * D], preferred_element_type=f32)
        x = x + mod_b[:, 0:D] * acc_s[...]
        h_b = _layernorm(x) * (1.0 + mod_b[:, 2 * D:3 * D]) + mod_b[:, D:2 * D]
        cp_b1.wait()
        cp_b2.wait()
        b1 = b1_v[...].astype(f32).reshape(1, F)
        b2 = b2_v[...].astype(f32).reshape(1, D)
        cp_w1.wait()
        g = jax.lax.dot_general(h_b.astype(bf), w1t_v[...], _NT,
                                preferred_element_type=f32) + b1
        g = jax.nn.gelu(g, approximate=True).astype(bf)
        y = jnp.broadcast_to(b2, (_ROWS, D))
        for cp, a, b in zip(cp_w2, w2_edges[:-1], w2_edges[1:]):
            cp.wait()
            y = y + jnp.dot(g[:, a:b], w2_v[a:b, :], preferred_element_type=f32)
        out = x + mod_b[:, 3 * D:4 * D] * y
        o_ref[...] = out[0:B].astype(o_ref.dtype)

    hbm = pl.BlockSpec(memory_space=pltpu.HBM)
    out = pl.pallas_call(
        kernel,
        out_shape=jax.ShapeDtypeStruct((B, D), A_x.dtype),
        in_specs=[hbm] * 11,
        out_specs=pl.BlockSpec(memory_space=pltpu.VMEM),
        scratch_shapes=[
            pltpu.VMEM((B, D), bf),
            pltpu.VMEM((B, D), bf),
            pltpu.VMEM((F,), bf),
            pltpu.VMEM((D,), bf),
            pltpu.VMEM((_NSLOT, B, W, Dh), bf),
            pltpu.VMEM((_NSLOT, B, W, Dh), bf),
            pltpu.VMEM((D, H * Dh), bf),
            pltpu.VMEM((H * Dh, D), bf),
            pltpu.VMEM((F, D), bf),
            pltpu.VMEM((F, D), bf),
            pltpu.VMEM((D, 6 * D), bf),
            pltpu.VMEM((H, _ROWS, Dh), f32),
            pltpu.VMEM((_ROWS, D), f32),
            pltpu.SemaphoreType.DMA((8 + n_w2,)),
            pltpu.SemaphoreType.DMA((_NSLOT,)),
            pltpu.SemaphoreType.DMA((_NSLOT,)),
        ],
        compiler_params=pltpu.CompilerParams(vmem_limit_bytes=48 * 1024 * 1024),
    )(A_x.reshape(B, D), c, B_b1, B_b2, A_k_cache, A_v_cache, A_wq, A_wo,
      B_w1.T, B_w2, w_mod)
    return out.reshape(B, Sq, D)
```
